```python
import os as _os
_os.environ.setdefault("JAX_PLATFORMS", "cpu")
import jax
import jax.numpy as jnp

def _softmax(x, axis=-1):
    return jax.nn.softmax(x, axis=axis)
def _gelu(x):
    return jax.nn.gelu(x, approximate=True)
def _silu(x):
    return jax.nn.silu(x)
def _sigmoid(x):
    return jax.nn.sigmoid(x)
def _layernorm(x, axis=-1, eps=1e-5):
    m = jnp.mean(x, axis=axis, keepdims=True)
    v = jnp.var(x, axis=axis, keepdims=True)
    return (x - m) / jnp.sqrt(v + eps)
def _scatter_add(tgt, idx, src, axis=0):
    return tgt.at[idx].add(src)
def _segment_sum(src, seg, n):
    return jax.ops.segment_sum(src, seg, n)
class _Rng:
    def __init__(self, key):
        self._k = key
    def _next(self):
        self._k, sub = jax.random.split(self._k)
        return sub
    def normal(self, shape):
        return jax.random.normal(self._next(), shape, dtype=jnp.bfloat16)
    def randint(self, lo, hi, shape):
        return jax.random.randint(self._next(), shape, lo, hi, dtype=jnp.int32)
    def uniform(self, shape, lo=0.0, hi=1.0):
        return jax.random.uniform(self._next(), shape, jnp.bfloat16, lo, hi)
    def permutation(self, n):
        return jax.random.permutation(self._next(), n)


kernel_name = 'sequential_preLN__sliding_local_dilated__dense_activation_mish__prompt'

def setup_inputs():
    _rng = _Rng(jax.random.key(int.from_bytes(__import__("os").urandom(4), "little")))
    _w = (lambda a: (lambda t: t.astype(jnp.bfloat16) if jnp.issubdtype(t.dtype, jnp.floating) else t)(jnp.asarray(a)))
    def _A_setup():
        B, S, D = 1, 2048, 512
        return {
            "x": _w((lambda *s: _rng.normal(s) * 0.05)(B, S, D)),
            "wqkv": _w((lambda *s: _rng.normal(s) * 0.05)(D, 3 * D)),
            "wo": _w((lambda *s: _rng.normal(s) * 0.05)(D, D)),
        }
    _A_in = _A_setup()

    def _B_setup():
        B, S, D, F = 1, 2048, 512, 1376
        return {
            "x": _w((lambda *s: _rng.normal(s) * 0.05)(B, S, D)),
            "w1": _w((lambda *s: _rng.normal(s) * 1.6)(D, F) * (D ** -0.5)),
            "b1": _w((lambda *s: _rng.normal(s) * 0.1)(F)),
            "w2": _w((lambda *s: _rng.normal(s) * 0.1)(F, D) * (F ** -0.5)),
        }
    _B_in = _B_setup()

    return {
        "A_x": _A_in["x"],
        "A_wqkv": _A_in["wqkv"],
        "A_wo": _A_in["wo"],
        "B_x": _B_in["x"],
        "B_w1": _B_in["w1"],
        "B_b1": _B_in["b1"],
        "B_w2": _B_in["w2"],
    }

def reference(A_x, A_wqkv, A_wo, B_x, B_w1, B_b1, B_w2):
    def _A_ref(x, wqkv, wo):
        B, S, D = x.shape
        H = 32; Dh = D // H
        W, dil = 8, 2
        qkv = (lambda x, *d: x.transpose(*d))((x @ wqkv).reshape(B, S, 3, H, Dh), 2, 0, 3, 1, 4)
        q, k, v = qkv[0], qkv[1], qkv[2]
        scale = Dh ** -0.5
        pos = jnp.arange(S)
        off = jnp.arange(W) * dil
        idx = pos[:, None] - off[None, :]
        mask = idx >= 0
        idx_c = jnp.where(mask, idx, 0).reshape(-1)
        kg = k[:, :, idx_c, :].reshape(B, H, S, W, Dh)
        vg = v[:, :, idx_c, :].reshape(B, H, S, W, Dh)
        logits = jnp.einsum("bhsd,bhswd->bhsw", q, kg) * scale
        logits = jnp.where(mask[None, None, :, :], logits, -1e9)
        attn = _softmax(logits, axis=-1)
        o = jnp.einsum("bhsw,bhswd->bhsd", attn, vg)
        return (lambda x, *d: x.transpose(*d))(o, 0, 2, 1, 3).reshape(B, S, D) @ wo

    def _B_ref(x, w1, b1, w2):
        h = jnp.einsum("bsd,df->bsf", x, w1) + b1
        sp = jnp.log1p(jnp.exp(-jnp.abs(h))) + jnp.where(h > 0, h, jnp.zeros_like(h))
        act = h * jnp.tanh(sp)
        return jnp.einsum("bsf,fd->bsd", act, w2)

    x = A_x
    h = x + _A_ref(_layernorm(x, axis=-1), A_wqkv, A_wo)
    h2 = h + _B_ref(_layernorm(h, axis=-1), B_w1, B_b1, B_w2)
    return h2
```

```python
import jax
import jax.numpy as jnp
import jax.experimental.pallas as pl
import jax.experimental.pallas.tpu as pltpu

S, D, F = 2048, 512, 1376
WINDOW, DILATION = 8, 2
R = 256
RW = R // 2
NT = S // R
G = 8
NG = R // G
HALO = 16
PB = 32
LOG2E = 1.4426950408889634
QK_SCALE = 0.25 * LOG2E
MASKED = -1e9 * LOG2E
f32, bf16, u32 = jnp.float32, jnp.bfloat16, jnp.uint32

_DMA_GROUPS = (("x01",), ("wq",), ("wk", "wv"), ("wo", "b1", "x2", "w1"), ("w2", "x37"))


def _att(t, chain, lag, tie, span, skip, pin=False):
    return ("att", t, dict(chain=chain, lag=lag, tie=tie, span=span, skip=skip, pin=pin))


_PROLOGUE = (
    ("wait", 0, None), ("ln", 0, None), ("ln", 1, None),
    ("wait", 1, None), ("perm_qkv", 0, None), ("q", 0, (0, 4)), ("q", 1, (0, 3)),
    ("wait", 2, None), ("perm_qkv", 1, None), ("q", 1, (3, 4)), ("k", 0, (0, 4)),
    ("perm_qkv", 2, None), ("v", 0, (0, 4)), ("k", 1, (0, 4)), ("v", 1, (0, 3)),
    _att(0, 7, 1, 2, 75, 10),
    ("wait", 3, None), ("v", 1, (3, 4)), ("perm_wo", 0, None), ("o", 0, None), ("ln", 2, None),
    ("q", 2, (0, 4)), ("k", 2, (0, 4)), ("v", 2, (0, 4)), ("prep_b", 0, None),
    _att(1, 8, 1, 3, 90, 5), ("o", 1, None), ("up", 0, None), ("mish", 0, None),
    ("wait", 4, None),
)
_BODY = (
    ("down", -2, None), ("ln", 1, None), ("q", 1, (0, 4)), ("k", 1, (0, 4)),
    _att(0, 7, 2, 3, 95, 0), ("o", 0, None), ("up", -1, None), ("mish", -1, None), ("v", 1, (0, 4)),
    ("ln", 2, None), ("down", -1, None), ("q", 2, (0, 4)), ("k", 2, (0, 4)),
    _att(1, 6, 0, 3, 85, 0), ("o", 1, None), ("up", 0, None), ("mish", 0, None), ("v", 2, (0, 4)),
    ("send", -2, 2),
)
_EPILOGUE = (
    ("down", 4, None), ("ln", 7, None), ("q", 7, (0, 4)), ("k", 7, (0, 4)),
    _att(6, 7, 1, 3, 90, 0), ("o", 6, None), ("v", 7, (0, 4)), ("up", 5, None), ("mish", 5, None),
    ("down", 5, None), _att(7, 8, 1, 2, 80, 10, pin=True), ("o", 7, None),
    ("up", 6, None), ("mish", 6, None), ("down", 6, None), ("up", 7, None),
    ("send", 4, 3), ("mish", 7, None), ("down", 7, None), ("send", 7, 1),
)
_LOOP_BASES = (2, 4)

_READS = dict(q=("xn",), k=("xn",), v=("xn",), o=("ctx",), up=("hn",), mish=("f",), down=("act", "h"))
_WRITES = dict(ln=("xn",), att=("ctx",), o=("h", "hn"), up=("f",), mish=("act",))


def _values_crossing_regions():
    regions = [("pro", _PROLOGUE, 0)] + [("body", _BODY, b) for b in _LOOP_BASES] + [("epi", _EPILOGUE, 0)]
    made, keep = {}, set()
    for idx, (region, steps, base) in enumerate(regions):
        for kind, off, _ in steps:
            for name in _READS.get(kind, ()):
                src_idx, src = made[name, base + off]
                if src_idx != idx:
                    keep.add(src)
            for name in _WRITES.get(kind, ()):
                made[name, base + off] = (idx, (region, kind, off, name))
    return frozenset(keep)


def _layernorm(x):
    m = jnp.mean(x, axis=-1, keepdims=True)
    c = x - m
    v = jnp.mean(c * c, axis=-1, keepdims=True)
    return c * jax.lax.rsqrt(v + 1e-5)


def _body(x_hbm, wqkv_hbm, wo_hbm, w1_hbm, b1_hbm, w2_hbm, out_hbm,
          x_v, wqkv_raw, wqkv_p, wo_raw, wo_p, w1_v, w2_v, b1_v, b1_f, out_v,
          k_s, v_s, q_s, h_s, hn_s, act_s, in_sem, out_sem):
    keep = _values_crossing_regions()
    stash = dict(h=h_s, hn=hn_s, act=act_s)

    def x_copy(t0, t1, sem):
        rows = pl.ds(t0 * R, (t1 - t0) * R)
        return pltpu.make_async_copy(x_hbm.at[rows, :], x_v.at[rows, :], sem)

    sem_of = {name: in_sem.at[i] for i, group in enumerate(_DMA_GROUPS) for name in group}
    copies = {
        "x01": x_copy(0, 2, sem_of["x01"]),
        "wq": pltpu.make_async_copy(wqkv_hbm.at[:, pl.ds(0, D)], wqkv_raw.at[0], sem_of["wq"]),
        "wk": pltpu.make_async_copy(wqkv_hbm.at[:, pl.ds(D, D)], wqkv_raw.at[1], sem_of["wk"]),
        "wv": pltpu.make_async_copy(wqkv_hbm.at[:, pl.ds(2 * D, D)], wqkv_raw.at[2], sem_of["wv"]),
        "wo": pltpu.make_async_copy(wo_hbm, wo_raw, sem_of["wo"]),
        "b1": pltpu.make_async_copy(b1_hbm, b1_v, sem_of["b1"]),
        "x2": x_copy(2, 3, sem_of["x2"]),
        "w1": pltpu.make_async_copy(w1_hbm, w1_v, sem_of["w1"]),
        "w2": pltpu.make_async_copy(w2_hbm, w2_v, sem_of["w2"]),
        "x37": x_copy(3, NT, sem_of["x37"]),
    }
    for group in _DMA_GROUPS:
        for name in group:
            copies[name].start()

    def out_copy(t0, tiles):
        rows = pl.ds(t0 * R, tiles * R)
        return pltpu.make_async_copy(out_v.at[rows, :], out_hbm.at[rows, :], out_sem.at[0])

    lane = jax.lax.broadcasted_iota(jnp.int32, (PB, 128), 1)
    lane_grp = (lane % 16) // 4
    lane_head = lane % 32

    def perm_qkv(p):
        src = wqkv_raw.at[p]
        idx = [(lane_head % 8) * 16 + 4 * ((lane_head // 8 + j) % 4) + lane // 32 for j in range(4)]
        for r0 in range(0, D // 2, PB):
            cols = [pltpu.bitcast(src[2 * r0:2 * (r0 + PB), i * 128:(i + 1) * 128], u32) for i in range(4)]
            for j in range(4):
                merged = cols[0]
                for i in range(1, 4):
                    merged = jnp.where(lane_grp == (i + j) % 4, cols[i], merged)
                wqkv_p[p, r0:r0 + PB, j * 128:(j + 1) * 128] = jnp.take_along_axis(merged, idx[j], axis=1)

    def perm_wo():
        sub = jax.lax.broadcasted_iota(jnp.int32, (8, 128), 0)

        def transpose8(xs):
            for b in (4, 2, 1):
                low = (sub & b) == 0
                ys = list(xs)
                for i in range(8):
                    if i & b == 0:
                        ys[i] = jnp.where(low, xs[i], pltpu.roll(xs[i + b], b, axis=0))
                        ys[i + b] = jnp.where(low, pltpu.roll(xs[i], 8 - b, axis=0), xs[i + b])
                xs = ys
            return xs

        for j in range(4):
            for a0 in (0, 8):
                even, odd = [], []
                for a in range(a0, a0 + 8):
                    lo = pltpu.bitcast(wo_raw[(2 * a) * 16:(2 * a) * 16 + 16, j * 128:(j + 1) * 128], u32)
                    hi = pltpu.bitcast(wo_raw[(2 * a + 1) * 16:(2 * a + 1) * 16 + 16, j * 128:(j + 1) * 128], u32)
                    even.append((lo & jnp.uint32(0xFFFF)) | (hi << 16))
                    odd.append((lo >> 16) | (hi & jnp.uint32(0xFFFF0000)))
                even, odd = transpose8(even), transpose8(odd)
                by_d = [None] * 16
                for m in range(8):
                    by_d[2 * m], by_d[2 * m + 1] = even[m], odd[m]
                i0 = a0 // 4
                for jj in range(4):
                    for g in range(4):
                        first = by_d[4 * ((i0 + jj) % 4) + g]
                        second = by_d[4 * ((i0 + 1 + jj) % 4) + g]
                        r = jj * 64 + g * 16 + a0
                        wo_p[r:r + 8, j * 128:(j + 1) * 128] = jnp.where(sub < 4, first, second)

    def prep_b():
        b1_f[...] = jnp.broadcast_to(b1_v[...].astype(f32)[None, :], (8, F))

    def weights(ref):
        return ref[...] if ref.dtype == bf16 else pltpu.bitcast(ref[...], bf16)

    def run_region(region, steps, base):
        local = {}
        matmuls = []
        att_parts = [None]

        def put(kind, name, off, val):
            local[name, off] = val
            if (region, kind, off, name) in keep:
                stash[name][base + off] = val if name == "h" else pltpu.bitcast(val, u32)

        def get(name, off):
            if (name, off) in local:
                return local[name, off]
            val = stash[name][base + off]
            return val if name == "h" else pltpu.bitcast(val, bf16)

        def matmul(lhs, rhs, cycles, transposed=False):
            dims = (((1,), (1 if transposed else 0,)), ((), ()))
            val = jax.lax.dot_general(lhs, rhs, dims, preferred_element_type=f32)
            matmuls.append((val, cycles))
            return val

        def first_row(t):
            return t * R if isinstance(t, int) else pl.multiple_of(t * R, R)

        def load_x(t):
            return x_v[pl.ds(first_row(t), R), :].astype(f32)

        def qkv_proj(kind, off, cols):
            t, (n0, n1), p = base + off, cols, "qkv".index(kind)
            first = isinstance(t, int) and t == 0
            last = isinstance(t, int) and t == NT - 1
            w = pltpu.bitcast(wqkv_p[p, :, n0 * 128:n1 * 128], bf16)
            val = matmul(get("xn", off), w, 8)
            if kind == "q":
                q_s[t, :, n0 * 128:n1 * 128] = val
                return
            dst = k_s if kind == "k" else v_s
            for j in range(n0, n1):
                col = val[:, (j - n0) * 128:(j - n0 + 1) * 128]
                dst[t, j, HALO:, :] = col
                if first:
                    dst[t, j, 0:HALO, :] = (jnp.zeros((HALO, 128), f32) if kind == "k"
                                            else jnp.broadcast_to(col[0:1, :], (HALO, 128)))
                if not last:
                    dst[t + 1, j, 0:HALO, :] = col[R - HALO:, :]

        def attention(off, opt):
            t = base + off
            first = isinstance(t, int) and t == 0
            stream, now = [], 0
            for val, cycles in matmuls[-opt["tie"]:]:
                for j in range(val.shape[1] // 128):
                    for r in range(R // 8):
                        stream.append((now, val, r, j))
                        now += cycles
            skip, span = opt["skip"] * now // 100, opt["span"] * now // 100
            release = []
            for g in range(NG):
                _, val, r, j = [e for e in stream if e[0] <= skip + g * span // NG][-1]
                release.append(val[r * 8:(r + 1) * 8, j * 128:(j + 1) * 128])

            denom, half, logits, ctx = [None] * NG, [None] * NG, [None] * NG, [None] * NG

            def products(g):
                r0 = g * G
                scale = jnp.full((G, 128), QK_SCALE, f32)
                if g >= opt["chain"]:
                    scale = jnp.minimum(scale, denom[g - opt["chain"]])
                gate = jnp.minimum(release[g], 0.0)
                if opt["pin"] and ("hn32", off - 1) in local:
                    gate = jnp.minimum(gate, local["hn32", off - 1][r0:r0 + 8, 0:128])
                scale = jnp.maximum(scale, gate)
                q = [q_s[t, r0:r0 + G, j * 128:(j + 1) * 128] * scale for j in range(4)]
                sums = []
                for w in range(WINDOW):
                    acc = None
                    for j in range(4):
                        prod = q[j] * k_s[t, j, pl.ds(HALO + r0 - w * DILATION, G), :]
                        acc = prod if acc is None else acc + prod
                    sums.append(acc)
                rolled = [pltpu.roll(s, 64, axis=1) for s in sums]
                half[g] = [s + r for s, r in zip(sums, rolled)]

            def finish_logits(g):
                r0 = g * G
                rolled = [pltpu.roll(s, 32, axis=1) for s in half[g]]
                full = [s + r for s, r in zip(half[g], rolled)]
                if first:
                    for w in range(WINDOW):
                        if r0 < w * DILATION:
                            pos = r0 + jax.lax.broadcasted_iota(jnp.int32, (G, 128), 0)
                            full[w] = jnp.where(pos >= w * DILATION, full[w], MASKED)
                logits[g] = full

            def softmax_values(g):
                r0 = g * G
                ls = logits[g]
                m = jnp.maximum(jnp.maximum(jnp.maximum(ls[0], ls[1]), jnp.maximum(ls[2], ls[3])),
                                jnp.maximum(jnp.maximum(ls[4], ls[5]), jnp.maximum(ls[6], ls[7])))
                es = [jnp.exp2(l - m) for l in ls]
                denom[g] = ((es[0] + es[1]) + (es[2] + es[3])) + ((es[4] + es[5]) + (es[6] + es[7]))
                acc = [None] * 4
                for w in range(WINDOW):
                    for j in range(4):
                        prod = es[w] * v_s[t, j, pl.ds(HALO + r0 - w * DILATION, G), :]
                        acc[j] = prod if acc[j] is None else acc[j] + prod
                inv = pltpu.reciprocal(denom[g], approx=True)
                ctx[g] = jnp.concatenate([a * inv for a in acc], axis=1)

            lag = opt["lag"]
            for i in range(NG + lag + 1):
                if i < NG:
                    products(i)
                if 0 <= i - lag < NG:
                    finish_logits(i - lag)
                if 0 <= i - lag - 1 < NG:
                    softmax_values(i - lag - 1)
            put("att", "ctx", off, jnp.concatenate(ctx, axis=0).astype(bf16))

        for kind, off, opt in steps:
            if kind == "wait":
                for name in _DMA_GROUPS[off]:
                    copies[name].wait()
            elif kind == "send":
                out_copy(base + off, opt).start()
            elif kind == "perm_qkv":
                perm_qkv(off)
            elif kind == "perm_wo":
                perm_wo()
            elif kind == "prep_b":
                prep_b()
            elif kind == "ln":
                put(kind, "xn", off, _layernorm(load_x(base + off)).astype(bf16))
            elif kind in ("q", "k", "v"):
                qkv_proj(kind, off, opt)
            elif kind == "att":
                attention(off, opt)
            elif kind == "o":
                h = load_x(base + off) + matmul(get("ctx", off), weights(wo_p), 8)
                put(kind, "h", off, h)
                hn = _layernorm(h)
                local["hn32", off] = hn
                put(kind, "hn", off, hn.astype(bf16))
            elif kind == "up":
                put(kind, "f", off, matmul(get("hn", off), weights(w1_v), 8, transposed=True) + b1_f[0:1, :])
            elif kind == "mish":
                f = get("f", off)
                e = jnp.exp2(jnp.minimum(f, 20.0) * LOG2E)
                n = e * (e + 2.0)
                put(kind, "act", off, (f * (n * pltpu.reciprocal(n + 2.0, approx=True))).astype(bf16))
            elif kind == "down":
                out = get("h", off) + matmul(get("act", off), weights(w2_v), 22)
                out_v[pl.ds(first_row(base + off), R), :] = out.astype(bf16)
            else:
                raise ValueError(kind)

    run_region("pro", _PROLOGUE, 0)

    def loop_step(k, carry):
        run_region("body", _BODY, _LOOP_BASES[0] + 2 * k)
        return carry

    jax.lax.fori_loop(0, len(_LOOP_BASES), loop_step, None)
    run_region("epi", _EPILOGUE, 0)

    for kind, off, opt in _EPILOGUE:
        if kind == "send":
            out_copy(off, opt).wait()
    for kind, off, opt in _BODY:
        if kind == "send":
            for b in _LOOP_BASES:
                out_copy(b + off, opt).wait()


def kernel(A_x, A_wqkv, A_wo, B_x, B_w1, B_b1, B_w2):
    del B_x
    hbm = pl.BlockSpec(memory_space=pltpu.HBM)
    out = pl.pallas_call(
        _body,
        in_specs=[hbm] * 6,
        out_specs=hbm,
        out_shape=jax.ShapeDtypeStruct((S, D), bf16),
        scratch_shapes=[
            pltpu.VMEM((S, D), bf16),
            pltpu.VMEM((3, D, D), bf16),
            pltpu.VMEM((3, D // 2, D), u32),
            pltpu.VMEM((D, D), bf16),
            pltpu.VMEM((D // 2, D), u32),
            pltpu.VMEM((F, D), bf16),
            pltpu.VMEM((F, D), bf16),
            pltpu.VMEM((F,), bf16),
            pltpu.VMEM((8, F), f32),
            pltpu.VMEM((S, D), bf16),
            pltpu.VMEM((NT, 4, HALO + R, 128), f32),
            pltpu.VMEM((NT, 4, HALO + R, 128), f32),
            pltpu.VMEM((NT, R, D), f32),
            pltpu.VMEM((NT, R, D), f32),
            pltpu.VMEM((NT, RW, D), u32),
            pltpu.VMEM((NT, RW, F), u32),
            pltpu.SemaphoreType.DMA((len(_DMA_GROUPS),)),
            pltpu.SemaphoreType.DMA((1,)),
        ],
        compiler_params=pltpu.CompilerParams(vmem_limit_bytes=100 * 1024 * 1024),
    )(A_x.reshape(S, D), A_wqkv, A_wo, B_w1.T, B_b1, B_w2)
    return out.reshape(1, S, D)


@jax.jit
def pallas_sequential_preLN__sliding_local_dilated__dense_activation_mish__prompt_kernel(
    A_x: jax.Array,
    A_wqkv: jax.Array,
    A_wo: jax.Array,
    B_x: jax.Array,
    B_w1: jax.Array,
    B_b1: jax.Array,
    B_w2: jax.Array,
):
    return kernel(A_x, A_wqkv, A_wo, B_x, B_w1, B_b1, B_w2)
```

```python
import jax
import jax.numpy as jnp
import jax.experimental.pallas as pl
import jax.experimental.pallas.tpu as pltpu

S, D, F = 2048, 512, 1376
WINDOW, DILATION = 8, 2
R = 256
RW = R // 2
NT = S // R
G = 8
NG = R // G
HALO = 16
PB = 32
LOG2E = 1.4426950408889634
QK_SCALE = 0.25 * LOG2E
MASKED = -1e9 * LOG2E
f32, bf16, u32 = jnp.float32, jnp.bfloat16, jnp.uint32

_DMA_GROUPS = (("x01",), ("wq",), ("wk", "wv"), ("wo", "b1", "x2", "w1"), ("w2", "x37"))


def _att(t, chain, lag, tie, span, skip, pin=False):
    return ("att", t, dict(chain=chain, lag=lag, tie=tie, span=span, skip=skip, pin=pin))


_PROLOGUE = (
    ("wait", 0, None), ("ln", 0, None), ("ln", 1, None),
    ("wait", 1, None), ("perm_qkv", 0, None), ("q", 0, (0, 4)), ("q", 1, (0, 3)),
    ("wait", 2, None), ("perm_qkv", 1, None), ("q", 1, (3, 4)), ("k", 0, (0, 4)),
    ("perm_qkv", 2, None), ("v", 0, (0, 4)), ("k", 1, (0, 4)),
    _att(0, 6, 2, 2, 85, 15), ("v", 1, (0, 3)),
    ("wait", 3, None), ("v", 1, (3, 4)), ("ln", 2, None), ("perm_wo", 0, None), ("o", 0, None),
    ("q", 2, (0, 4)), ("prep_b", 0, None), ("v", 2, (0, 3)), ("k", 2, (0, 4)),
    _att(1, 5, 1, 4, 80, 5), ("o", 1, None), ("v", 2, (3, 4)), ("up", 0, None), ("mish", 0, None),
    ("wait", 4, None),
)
_BODY = (
    ("down", -2, None), ("ln", 1, None), ("q", 1, (0, 4)), ("k", 1, (0, 4)),
    _att(0, 7, 2, 3, 98, 0), ("o", 0, None), ("up", -1, None), ("v", 1, (0, 4)),
    ("ln", 2, None), ("mish", -1, None), ("down", -1, None), ("q", 2, (0, 4)), ("k", 2, (0, 4)),
    _att(1, 6, 0, 3, 85, 0), ("o", 1, None), ("up", 0, None), ("mish", 0, None), ("v", 2, (0, 4)),
    ("send", -2, 2),
)
_EPILOGUE = (
    ("down", 4, None), ("ln", 7, None), ("q", 7, (0, 4)), ("k", 7, (0, 4)),
    _att(6, 5, 2, 3, 98, 0), ("o", 6, None), ("v", 7, (0, 4)), ("up", 5, None), ("mish", 5, None),
    ("down", 5, None), _att(7, 9, 1, 2, 80, 10, pin=True), ("o", 7, None),
    ("up", 6, None), ("mish", 6, None), ("down", 6, None), ("up", 7, None),
    ("send", 4, 3), ("mish", 7, None), ("down", 7, None), ("send", 7, 1),
)
_LOOP_BASES = (2, 4)

_READS = dict(q=("xn",), k=("xn",), v=("xn",), o=("ctx",), up=("hn",), mish=("f",), down=("act", "h"))
_WRITES = dict(ln=("xn",), att=("ctx",), o=("h", "hn"), up=("f",), mish=("act",))


def _values_crossing_regions():
    regions = [("pro", _PROLOGUE, 0)] + [("body", _BODY, b) for b in _LOOP_BASES] + [("epi", _EPILOGUE, 0)]
    made, keep = {}, set()
    for idx, (region, steps, base) in enumerate(regions):
        for kind, off, _ in steps:
            for name in _READS.get(kind, ()):
                src_idx, src = made[name, base + off]
                if src_idx != idx:
                    keep.add(src)
            for name in _WRITES.get(kind, ()):
                made[name, base + off] = (idx, (region, kind, off, name))
    return frozenset(keep)


def _layernorm(x):
    m = jnp.mean(x, axis=-1, keepdims=True)
    c = x - m
    v = jnp.mean(c * c, axis=-1, keepdims=True)
    return c * jax.lax.rsqrt(v + 1e-5)


def _body(x_hbm, wqkv_hbm, wo_hbm, w1_hbm, b1_hbm, w2_hbm, out_hbm,
          x_v, wqkv_raw, wqkv_p, wo_raw, wo_p, w1_v, w2_v, b1_v, b1_f, out_v,
          k_s, v_s, q_s, h_s, hn_s, act_s, in_sem, out_sem):
    keep = _values_crossing_regions()
    stash = dict(h=h_s, hn=hn_s, act=act_s)

    def x_copy(t0, t1, sem):
        rows = pl.ds(t0 * R, (t1 - t0) * R)
        return pltpu.make_async_copy(x_hbm.at[rows, :], x_v.at[rows, :], sem)

    sem_of = {name: in_sem.at[i] for i, group in enumerate(_DMA_GROUPS) for name in group}
    copies = {
        "x01": x_copy(0, 2, sem_of["x01"]),
        "wq": pltpu.make_async_copy(wqkv_hbm.at[:, pl.ds(0, D)], wqkv_raw.at[0], sem_of["wq"]),
        "wk": pltpu.make_async_copy(wqkv_hbm.at[:, pl.ds(D, D)], wqkv_raw.at[1], sem_of["wk"]),
        "wv": pltpu.make_async_copy(wqkv_hbm.at[:, pl.ds(2 * D, D)], wqkv_raw.at[2], sem_of["wv"]),
        "wo": pltpu.make_async_copy(wo_hbm, wo_raw, sem_of["wo"]),
        "b1": pltpu.make_async_copy(b1_hbm, b1_v, sem_of["b1"]),
        "x2": x_copy(2, 3, sem_of["x2"]),
        "w1": pltpu.make_async_copy(w1_hbm, w1_v, sem_of["w1"]),
        "w2": pltpu.make_async_copy(w2_hbm, w2_v, sem_of["w2"]),
        "x37": x_copy(3, NT, sem_of["x37"]),
    }
    for group in _DMA_GROUPS:
        for name in group:
            copies[name].start()

    def out_copy(t0, tiles):
        rows = pl.ds(t0 * R, tiles * R)
        return pltpu.make_async_copy(out_v.at[rows, :], out_hbm.at[rows, :], out_sem.at[0])

    lane = jax.lax.broadcasted_iota(jnp.int32, (PB, 128), 1)
    lane_grp = (lane % 16) // 4
    lane_head = lane % 32

    def perm_qkv(p):
        src = wqkv_raw.at[p]
        idx = [(lane_head % 8) * 16 + 4 * ((lane_head // 8 + j) % 4) + lane // 32 for j in range(4)]
        for r0 in range(0, D // 2, PB):
            cols = [pltpu.bitcast(src[2 * r0:2 * (r0 + PB), i * 128:(i + 1) * 128], u32) for i in range(4)]
            for j in range(4):
                merged = cols[0]
                for i in range(1, 4):
                    merged = jnp.where(lane_grp == (i + j) % 4, cols[i], merged)
                wqkv_p[p, r0:r0 + PB, j * 128:(j + 1) * 128] = jnp.take_along_axis(merged, idx[j], axis=1)

    def perm_wo():
        sub = jax.lax.broadcasted_iota(jnp.int32, (8, 128), 0)

        def transpose8(xs):
            for b in (4, 2, 1):
                low = (sub & b) == 0
                ys = list(xs)
                for i in range(8):
                    if i & b == 0:
                        ys[i] = jnp.where(low, xs[i], pltpu.roll(xs[i + b], b, axis=0))
                        ys[i + b] = jnp.where(low, pltpu.roll(xs[i], 8 - b, axis=0), xs[i + b])
                xs = ys
            return xs

        for j in range(4):
            for a0 in (0, 8):
                even, odd = [], []
                for a in range(a0, a0 + 8):
                    lo = pltpu.bitcast(wo_raw[(2 * a) * 16:(2 * a) * 16 + 16, j * 128:(j + 1) * 128], u32)
                    hi = pltpu.bitcast(wo_raw[(2 * a + 1) * 16:(2 * a + 1) * 16 + 16, j * 128:(j + 1) * 128], u32)
                    even.append((lo & jnp.uint32(0xFFFF)) | (hi << 16))
                    odd.append((lo >> 16) | (hi & jnp.uint32(0xFFFF0000)))
                even, odd = transpose8(even), transpose8(odd)
                by_d = [None] * 16
                for m in range(8):
                    by_d[2 * m], by_d[2 * m + 1] = even[m], odd[m]
                i0 = a0 // 4
                for jj in range(4):
                    for g in range(4):
                        first = by_d[4 * ((i0 + jj) % 4) + g]
                        second = by_d[4 * ((i0 + 1 + jj) % 4) + g]
                        r = jj * 64 + g * 16 + a0
                        wo_p[r:r + 8, j * 128:(j + 1) * 128] = jnp.where(sub < 4, first, second)

    def prep_b():
        b1_f[...] = jnp.broadcast_to(b1_v[...].astype(f32)[None, :], (8, F))

    def weights(ref):
        return ref[...] if ref.dtype == bf16 else pltpu.bitcast(ref[...], bf16)

    def run_region(region, steps, base):
        local = {}
        matmuls = []
        att_parts = [None]

        def put(kind, name, off, val):
            local[name, off] = val
            if (region, kind, off, name) in keep:
                stash[name][base + off] = val if name == "h" else pltpu.bitcast(val, u32)

        def get(name, off):
            if (name, off) in local:
                return local[name, off]
            val = stash[name][base + off]
            return val if name == "h" else pltpu.bitcast(val, bf16)

        def matmul(lhs, rhs, cycles, transposed=False):
            dims = (((1,), (1 if transposed else 0,)), ((), ()))
            val = jax.lax.dot_general(lhs, rhs, dims, preferred_element_type=f32)
            matmuls.append((val, cycles))
            return val

        def first_row(t):
            return t * R if isinstance(t, int) else pl.multiple_of(t * R, R)

        def load_x(t):
            return x_v[pl.ds(first_row(t), R), :].astype(f32)

        def qkv_proj(kind, off, cols):
            t, (n0, n1), p = base + off, cols, "qkv".index(kind)
            first = isinstance(t, int) and t == 0
            last = isinstance(t, int) and t == NT - 1
            w = pltpu.bitcast(wqkv_p[p, :, n0 * 128:n1 * 128], bf16)
            val = matmul(get("xn", off), w, 8)
            if kind == "q":
                q_s[t, :, n0 * 128:n1 * 128] = val
                return
            dst = k_s if kind == "k" else v_s
            for j in range(n0, n1):
                col = val[:, (j - n0) * 128:(j - n0 + 1) * 128]
                dst[t, j, HALO:, :] = col
                if first:
                    dst[t, j, 0:HALO, :] = (jnp.zeros((HALO, 128), f32) if kind == "k"
                                            else jnp.broadcast_to(col[0:1, :], (HALO, 128)))
                if not last:
                    dst[t + 1, j, 0:HALO, :] = col[R - HALO:, :]

        def attention(off, opt):
            t = base + off
            first = isinstance(t, int) and t == 0
            stream, now = [], 0
            for val, cycles in matmuls[-opt["tie"]:]:
                for j in range(val.shape[1] // 128):
                    for r in range(R // 8):
                        stream.append((now, val, r, j))
                        now += cycles
            skip, span = opt["skip"] * now // 100, opt["span"] * now // 100
            release = []
            for g in range(NG):
                _, val, r, j = [e for e in stream if e[0] <= skip + g * span // NG][-1]
                release.append(val[r * 8:(r + 1) * 8, j * 128:(j + 1) * 128])

            denom, half, logits, ctx = [None] * NG, [None] * NG, [None] * NG, [None] * NG

            def products(g):
                r0 = g * G
                scale = jnp.full((G, 128), QK_SCALE, f32)
                if g >= opt["chain"]:
                    scale = jnp.minimum(scale, denom[g - opt["chain"]])
                gate = jnp.minimum(release[g], 0.0)
                if opt["pin"] and ("hn32", off - 1) in local:
                    gate = jnp.minimum(gate, local["hn32", off - 1][r0:r0 + 8, 0:128])
                scale = jnp.maximum(scale, gate)
                q = [q_s[t, r0:r0 + G, j * 128:(j + 1) * 128] * scale for j in range(4)]
                sums = []
                for w in range(WINDOW):
                    acc = None
                    for j in range(4):
                        prod = q[j] * k_s[t, j, pl.ds(HALO + r0 - w * DILATION, G), :]
                        acc = prod if acc is None else acc + prod
                    sums.append(acc)
                rolled = [pltpu.roll(s, 64, axis=1) for s in sums]
                half[g] = [s + r for s, r in zip(sums, rolled)]

            def finish_logits(g):
                r0 = g * G
                rolled = [pltpu.roll(s, 32, axis=1) for s in half[g]]
                full = [s + r for s, r in zip(half[g], rolled)]
                if first:
                    for w in range(WINDOW):
                        if r0 < w * DILATION:
                            pos = r0 + jax.lax.broadcasted_iota(jnp.int32, (G, 128), 0)
                            full[w] = jnp.where(pos >= w * DILATION, full[w], MASKED)
                logits[g] = full

            def softmax_values(g):
                r0 = g * G
                ls = logits[g]
                m = jnp.maximum(jnp.maximum(jnp.maximum(ls[0], ls[1]), jnp.maximum(ls[2], ls[3])),
                                jnp.maximum(jnp.maximum(ls[4], ls[5]), jnp.maximum(ls[6], ls[7])))
                es = [jnp.exp2(l - m) for l in ls]
                denom[g] = ((es[0] + es[1]) + (es[2] + es[3])) + ((es[4] + es[5]) + (es[6] + es[7]))
                acc = [None] * 4
                for w in range(WINDOW):
                    for j in range(4):
                        prod = es[w] * v_s[t, j, pl.ds(HALO + r0 - w * DILATION, G), :]
                        acc[j] = prod if acc[j] is None else acc[j] + prod
                inv = pltpu.reciprocal(denom[g], approx=True)
                ctx[g] = jnp.concatenate([a * inv for a in acc], axis=1)

            lag = opt["lag"]
            for i in range(NG + lag + 1):
                if i < NG:
                    products(i)
                if 0 <= i - lag < NG:
                    finish_logits(i - lag)
                if 0 <= i - lag - 1 < NG:
                    softmax_values(i - lag - 1)
            put("att", "ctx", off, jnp.concatenate(ctx, axis=0).astype(bf16))

        for kind, off, opt in steps:
            if kind == "wait":
                for name in _DMA_GROUPS[off]:
                    copies[name].wait()
            elif kind == "send":
                out_copy(base + off, opt).start()
            elif kind == "perm_qkv":
                perm_qkv(off)
            elif kind == "perm_wo":
                perm_wo()
            elif kind == "prep_b":
                prep_b()
            elif kind == "ln":
                put(kind, "xn", off, _layernorm(load_x(base + off)).astype(bf16))
            elif kind in ("q", "k", "v"):
                qkv_proj(kind, off, opt)
            elif kind == "att":
                attention(off, opt)
            elif kind == "o":
                h = load_x(base + off) + matmul(get("ctx", off), weights(wo_p), 8)
                put(kind, "h", off, h)
                hn = _layernorm(h)
                local["hn32", off] = hn
                put(kind, "hn", off, hn.astype(bf16))
            elif kind == "up":
                put(kind, "f", off, matmul(get("hn", off), weights(w1_v), 8, transposed=True) + b1_f[0:1, :])
            elif kind == "mish":
                f = get("f", off)
                e = jnp.exp2(jnp.minimum(f, 20.0) * LOG2E)
                n = e * (e + 2.0)
                put(kind, "act", off, (f * (n * pltpu.reciprocal(n + 2.0, approx=True))).astype(bf16))
            elif kind == "down":
                out = get("h", off) + matmul(get("act", off), weights(w2_v), 22)
                out_v[pl.ds(first_row(base + off), R), :] = out.astype(bf16)
            else:
                raise ValueError(kind)

    run_region("pro", _PROLOGUE, 0)

    def loop_step(k, carry):
        run_region("body", _BODY, _LOOP_BASES[0] + 2 * k)
        return carry

    jax.lax.fori_loop(0, len(_LOOP_BASES), loop_step, None)
    run_region("epi", _EPILOGUE, 0)

    for kind, off, opt in _EPILOGUE:
        if kind == "send":
            out_copy(off, opt).wait()
    for kind, off, opt in _BODY:
        if kind == "send":
            for b in _LOOP_BASES:
                out_copy(b + off, opt).wait()


def kernel(A_x, A_wqkv, A_wo, B_x, B_w1, B_b1, B_w2):
    del B_x
    hbm = pl.BlockSpec(memory_space=pltpu.HBM)
    out = pl.pallas_call(
        _body,
        in_specs=[hbm] * 6,
        out_specs=hbm,
        out_shape=jax.ShapeDtypeStruct((S, D), bf16),
        scratch_shapes=[
            pltpu.VMEM((S, D), bf16),
            pltpu.VMEM((3, D, D), bf16),
            pltpu.VMEM((3, D // 2, D), u32),
            pltpu.VMEM((D, D), bf16),
            pltpu.VMEM((D // 2, D), u32),
            pltpu.VMEM((F, D), bf16),
            pltpu.VMEM((F, D), bf16),
            pltpu.VMEM((F,), bf16),
            pltpu.VMEM((8, F), f32),
            pltpu.VMEM((S, D), bf16),
            pltpu.VMEM((NT, 4, HALO + R, 128), f32),
            pltpu.VMEM((NT, 4, HALO + R, 128), f32),
            pltpu.VMEM((NT, R, D), f32),
            pltpu.VMEM((NT, R, D), f32),
            pltpu.VMEM((NT, RW, D), u32),
            pltpu.VMEM((NT, RW, F), u32),
            pltpu.SemaphoreType.DMA((len(_DMA_GROUPS),)),
            pltpu.SemaphoreType.DMA((1,)),
        ],
        compiler_params=pltpu.CompilerParams(vmem_limit_bytes=100 * 1024 * 1024),
    )(A_x.reshape(S, D), A_wqkv, A_wo, B_w1.T, B_b1, B_w2)
    return out.reshape(1, S, D)


@jax.jit
def pallas_sequential_preLN__sliding_local_dilated__dense_activation_mish__prompt_kernel(
    A_x: jax.Array,
    A_wqkv: jax.Array,
    A_wo: jax.Array,
    B_x: jax.Array,
    B_w1: jax.Array,
    B_b1: jax.Array,
    B_w2: jax.Array,
):
    return kernel(A_x, A_wqkv, A_wo, B_x, B_w1, B_b1, B_w2)
```

```python
import jax
import jax.numpy as jnp
import jax.experimental.pallas as pl
import jax.experimental.pallas.tpu as pltpu

S, D, F = 2048, 512, 1376
WINDOW, DILATION = 8, 2
R = 256
RW = R // 2
NT = S // R
G = 8
NG = R // G
HALO = 16
PB = 32
LOG2E = 1.4426950408889634
QK_SCALE = 0.25 * LOG2E
MASKED = -1e9 * LOG2E
f32, bf16, u32 = jnp.float32, jnp.bfloat16, jnp.uint32

_DMA_GROUPS = (("x0",), ("wq",), ("x12",), ("wk", "wv"), ("wo", "b1", "w1"), ("w2", "x37"))


def _att(t, chain, lag, tie, span, skip, pin=False):
    return ("att", t, dict(chain=chain, lag=lag, tie=tie, span=span, skip=skip, pin=pin))


_PROLOGUE = (
    ("wait", 0, None), ("ln", 0, None),
    ("wait", 1, None), ("perm_qkv", 0, None), ("q", 0, (0, 2)),
    ("wait", 2, None), ("ln", 1, None), ("q", 0, (2, 4)), ("q", 1, (0, 4)), ("ln", 2, None), ("q", 2, (0, 3)),
    ("wait", 3, None), ("perm_qkv", 1, None), ("q", 2, (3, 4)), ("k", 0, (0, 4)),
    ("perm_qkv", 2, None), ("v", 0, (0, 4)), ("k", 1, (0, 4)),
    _att(0, 6, 2, 2, 85, 15), ("v", 1, (0, 3)),
    ("wait", 4, None), ("v", 1, (3, 4)), ("perm_wo", 0, None), ("o", 0, None), ("prep_b", 0, None),
    ("k", 2, (0, 4)), ("v", 2, (0, 3)),
    _att(1, 6, 1, 3, 90, 8), ("o", 1, None), ("up", 0, None), ("v", 2, (3, 4)), ("mish", 0, None),
    ("wait", 5, None),
)
_BODY = (
    ("down", -2, None), ("ln", 1, None), ("q", 1, (0, 4)), ("k", 1, (0, 4)),
    _att(0, 7, 2, 3, 98, 0), ("o", 0, None), ("up", -1, None), ("v", 1, (0, 4)),
    ("ln", 2, None), ("q", 2, (0, 4)), ("mish", -1, None), ("down", -1, None), ("k", 2, (0, 4)),
    _att(1, 6, 0, 3, 85, 0), ("o", 1, None), ("up", 0, None), ("mish", 0, None), ("v", 2, (0, 4)),
    ("send", -2, 2),
)
_EPILOGUE = (
    ("down", 4, None), ("ln", 7, None), ("q", 7, (0, 4)), ("k", 7, (0, 4)),
    _att(6, 5, 2, 3, 98, 0), ("o", 6, None), ("v", 7, (0, 4)), ("up", 5, None), ("mish", 5, None),
    _att(7, 9, 1, 2, 80, 10, pin=True), ("o", 7, None), ("down", 5, None),
    ("up", 6, None), ("mish", 6, None), ("down", 6, None), ("up", 7, None),
    ("send", 4, 3), ("mish", 7, None), ("down", 7, None), ("send", 7, 1),
)
_LOOP_BASES = (2, 4)

_READS = dict(q=("xn",), k=("xn",), v=("xn",), o=("ctx",), up=("hn",), mish=("f",), down=("act", "h"))
_WRITES = dict(ln=("xn",), att=("ctx",), o=("h", "hn"), up=("f",), mish=("act",))


def _values_crossing_regions():
    regions = [("pro", _PROLOGUE, 0)] + [("body", _BODY, b) for b in _LOOP_BASES] + [("epi", _EPILOGUE, 0)]
    made, keep = {}, set()
    for idx, (region, steps, base) in enumerate(regions):
        for kind, off, _ in steps:
            for name in _READS.get(kind, ()):
                src_idx, src = made[name, base + off]
                if src_idx != idx:
                    keep.add(src)
            for name in _WRITES.get(kind, ()):
                made[name, base + off] = (idx, (region, kind, off, name))
    return frozenset(keep)


def _layernorm(x):
    m = jnp.mean(x, axis=-1, keepdims=True)
    c = x - m
    v = jnp.mean(c * c, axis=-1, keepdims=True)
    return c * jax.lax.rsqrt(v + 1e-5)


def _body(x_hbm, wqkv_hbm, wo_hbm, w1_hbm, b1_hbm, w2_hbm, out_hbm,
          x_v, wqkv_raw, wqkv_p, wo_raw, wo_p, w1_v, w2_v, b1_v, b1_f, out_v,
          k_s, v_s, q_s, h_s, hn_s, act_s, in_sem, out_sem):
    keep = _values_crossing_regions()
    stash = dict(h=h_s, hn=hn_s, act=act_s)

    def x_copy(t0, t1, sem):
        rows = pl.ds(t0 * R, (t1 - t0) * R)
        return pltpu.make_async_copy(x_hbm.at[rows, :], x_v.at[rows, :], sem)

    sem_of = {name: in_sem.at[i] for i, group in enumerate(_DMA_GROUPS) for name in group}
    copies = {
        "x0": x_copy(0, 1, sem_of["x0"]),
        "wq": pltpu.make_async_copy(wqkv_hbm.at[:, pl.ds(0, D)], wqkv_raw.at[0], sem_of["wq"]),
        "wk": pltpu.make_async_copy(wqkv_hbm.at[:, pl.ds(D, D)], wqkv_raw.at[1], sem_of["wk"]),
        "wv": pltpu.make_async_copy(wqkv_hbm.at[:, pl.ds(2 * D, D)], wqkv_raw.at[2], sem_of["wv"]),
        "wo": pltpu.make_async_copy(wo_hbm, wo_raw, sem_of["wo"]),
        "b1": pltpu.make_async_copy(b1_hbm, b1_v, sem_of["b1"]),
        "x12": x_copy(1, 3, sem_of["x12"]),
        "w1": pltpu.make_async_copy(w1_hbm, w1_v, sem_of["w1"]),
        "w2": pltpu.make_async_copy(w2_hbm, w2_v, sem_of["w2"]),
        "x37": x_copy(3, NT, sem_of["x37"]),
    }
    for group in _DMA_GROUPS:
        for name in group:
            copies[name].start()

    def out_copy(t0, tiles):
        rows = pl.ds(t0 * R, tiles * R)
        return pltpu.make_async_copy(out_v.at[rows, :], out_hbm.at[rows, :], out_sem.at[0])

    lane = jax.lax.broadcasted_iota(jnp.int32, (PB, 128), 1)
    lane_grp = (lane % 16) // 4
    lane_head = lane % 32

    def perm_qkv(p):
        src = wqkv_raw.at[p]
        idx = [(lane_head % 8) * 16 + 4 * ((lane_head // 8 + j) % 4) + lane // 32 for j in range(4)]
        for r0 in range(0, D // 2, PB):
            cols = [pltpu.bitcast(src[2 * r0:2 * (r0 + PB), i * 128:(i + 1) * 128], u32) for i in range(4)]
            for j in range(4):
                merged = cols[0]
                for i in range(1, 4):
                    merged = jnp.where(lane_grp == (i + j) % 4, cols[i], merged)
                wqkv_p[p, r0:r0 + PB, j * 128:(j + 1) * 128] = jnp.take_along_axis(merged, idx[j], axis=1)

    def perm_wo():
        sub = jax.lax.broadcasted_iota(jnp.int32, (8, 128), 0)

        def transpose8(xs):
            for b in (4, 2, 1):
                low = (sub & b) == 0
                ys = list(xs)
                for i in range(8):
                    if i & b == 0:
                        ys[i] = jnp.where(low, xs[i], pltpu.roll(xs[i + b], b, axis=0))
                        ys[i + b] = jnp.where(low, pltpu.roll(xs[i], 8 - b, axis=0), xs[i + b])
                xs = ys
            return xs

        for j in range(4):
            for a0 in (0, 8):
                even, odd = [], []
                for a in range(a0, a0 + 8):
                    lo = pltpu.bitcast(wo_raw[(2 * a) * 16:(2 * a) * 16 + 16, j * 128:(j + 1) * 128], u32)
                    hi = pltpu.bitcast(wo_raw[(2 * a + 1) * 16:(2 * a + 1) * 16 + 16, j * 128:(j + 1) * 128], u32)
                    even.append((lo & jnp.uint32(0xFFFF)) | (hi << 16))
                    odd.append((lo >> 16) | (hi & jnp.uint32(0xFFFF0000)))
                even, odd = transpose8(even), transpose8(odd)
                by_d = [None] * 16
                for m in range(8):
                    by_d[2 * m], by_d[2 * m + 1] = even[m], odd[m]
                i0 = a0 // 4
                for jj in range(4):
                    for g in range(4):
                        first = by_d[4 * ((i0 + jj) % 4) + g]
                        second = by_d[4 * ((i0 + 1 + jj) % 4) + g]
                        r = jj * 64 + g * 16 + a0
                        wo_p[r:r + 8, j * 128:(j + 1) * 128] = jnp.where(sub < 4, first, second)

    def prep_b():
        b1_f[...] = jnp.broadcast_to(b1_v[...].astype(f32)[None, :], (8, F))

    def weights(ref):
        return ref[...] if ref.dtype == bf16 else pltpu.bitcast(ref[...], bf16)

    def run_region(region, steps, base):
        local = {}
        matmuls = []
        att_parts = [None]

        def put(kind, name, off, val):
            local[name, off] = val
            if (region, kind, off, name) in keep:
                stash[name][base + off] = val if name == "h" else pltpu.bitcast(val, u32)

        def get(name, off):
            if (name, off) in local:
                return local[name, off]
            val = stash[name][base + off]
            return val if name == "h" else pltpu.bitcast(val, bf16)

        def matmul(lhs, rhs, cycles, transposed=False):
            dims = (((1,), (1 if transposed else 0,)), ((), ()))
            val = jax.lax.dot_general(lhs, rhs, dims, preferred_element_type=f32)
            matmuls.append((val, cycles))
            return val

        def first_row(t):
            return t * R if isinstance(t, int) else pl.multiple_of(t * R, R)

        def load_x(t):
            return x_v[pl.ds(first_row(t), R), :].astype(f32)

        def qkv_proj(kind, off, cols):
            t, (n0, n1), p = base + off, cols, "qkv".index(kind)
            first = isinstance(t, int) and t == 0
            last = isinstance(t, int) and t == NT - 1
            w = pltpu.bitcast(wqkv_p[p, :, n0 * 128:n1 * 128], bf16)
            val = matmul(get("xn", off), w, 8)
            if kind == "q":
                q_s[t, :, n0 * 128:n1 * 128] = val
                return
            dst = k_s if kind == "k" else v_s
            for j in range(n0, n1):
                col = val[:, (j - n0) * 128:(j - n0 + 1) * 128]
                dst[t, j, HALO:, :] = col
                if first:
                    dst[t, j, 0:HALO, :] = (jnp.zeros((HALO, 128), f32) if kind == "k"
                                            else jnp.broadcast_to(col[0:1, :], (HALO, 128)))
                if not last:
                    dst[t + 1, j, 0:HALO, :] = col[R - HALO:, :]

        def attention(off, opt):
            t = base + off
            first = isinstance(t, int) and t == 0
            stream, now = [], 0
            for val, cycles in matmuls[-opt["tie"]:]:
                for j in range(val.shape[1] // 128):
                    for r in range(R // 8):
                        stream.append((now, val, r, j))
                        now += cycles
            skip, span = opt["skip"] * now // 100, opt["span"] * now // 100
            release = []
            for g in range(NG):
                _, val, r, j = [e for e in stream if e[0] <= skip + g * span // NG][-1]
                release.append(val[r * 8:(r + 1) * 8, j * 128:(j + 1) * 128])

            denom, half, logits, ctx = [None] * NG, [None] * NG, [None] * NG, [None] * NG

            def products(g):
                r0 = g * G
                scale = jnp.full((G, 128), QK_SCALE, f32)
                if g >= opt["chain"]:
                    scale = jnp.minimum(scale, denom[g - opt["chain"]])
                gate = jnp.minimum(release[g], 0.0)
                if opt["pin"] and ("hn32", off - 1) in local:
                    gate = jnp.minimum(gate, local["hn32", off - 1][r0:r0 + 8, 0:128])
                scale = jnp.maximum(scale, gate)
                q = [q_s[t, r0:r0 + G, j * 128:(j + 1) * 128] * scale for j in range(4)]
                sums = []
                for w in range(WINDOW):
                    acc = None
                    for j in range(4):
                        prod = q[j] * k_s[t, j, pl.ds(HALO + r0 - w * DILATION, G), :]
                        acc = prod if acc is None else acc + prod
                    sums.append(acc)
                rolled = [pltpu.roll(s, 64, axis=1) for s in sums]
                half[g] = [s + r for s, r in zip(sums, rolled)]

            def finish_logits(g):
                r0 = g * G
                rolled = [pltpu.roll(s, 32, axis=1) for s in half[g]]
                full = [s + r for s, r in zip(half[g], rolled)]
                if first:
                    for w in range(WINDOW):
                        if r0 < w * DILATION:
                            pos = r0 + jax.lax.broadcasted_iota(jnp.int32, (G, 128), 0)
                            full[w] = jnp.where(pos >= w * DILATION, full[w], MASKED)
                logits[g] = full

            def softmax_values(g):
                r0 = g * G
                ls = logits[g]
                m = jnp.maximum(jnp.maximum(jnp.maximum(ls[0], ls[1]), jnp.maximum(ls[2], ls[3])),
                                jnp.maximum(jnp.maximum(ls[4], ls[5]), jnp.maximum(ls[6], ls[7])))
                es = [jnp.exp2(l - m) for l in ls]
                denom[g] = ((es[0] + es[1]) + (es[2] + es[3])) + ((es[4] + es[5]) + (es[6] + es[7]))
                acc = [None] * 4
                for w in range(WINDOW):
                    for j in range(4):
                        prod = es[w] * v_s[t, j, pl.ds(HALO + r0 - w * DILATION, G), :]
                        acc[j] = prod if acc[j] is None else acc[j] + prod
                inv = pltpu.reciprocal(denom[g], approx=True)
                ctx[g] = jnp.concatenate([a * inv for a in acc], axis=1)

            lag = opt["lag"]
            for i in range(NG + lag + 1):
                if i < NG:
                    products(i)
                if 0 <= i - lag < NG:
                    finish_logits(i - lag)
                if 0 <= i - lag - 1 < NG:
                    softmax_values(i - lag - 1)
            put("att", "ctx", off, jnp.concatenate(ctx, axis=0).astype(bf16))

        for kind, off, opt in steps:
            if kind == "wait":
                for name in _DMA_GROUPS[off]:
                    copies[name].wait()
            elif kind == "send":
                out_copy(base + off, opt).start()
            elif kind == "perm_qkv":
                perm_qkv(off)
            elif kind == "perm_wo":
                perm_wo()
            elif kind == "prep_b":
                prep_b()
            elif kind == "ln":
                put(kind, "xn", off, _layernorm(load_x(base + off)).astype(bf16))
            elif kind in ("q", "k", "v"):
                qkv_proj(kind, off, opt)
            elif kind == "att":
                attention(off, opt)
            elif kind == "o":
                h = load_x(base + off) + matmul(get("ctx", off), weights(wo_p), 8)
                put(kind, "h", off, h)
                hn = _layernorm(h)
                local["hn32", off] = hn
                put(kind, "hn", off, hn.astype(bf16))
            elif kind == "up":
                put(kind, "f", off, matmul(get("hn", off), weights(w1_v), 8, transposed=True) + b1_f[0:1, :])
            elif kind == "mish":
                f = get("f", off)
                e = jnp.exp2(jnp.minimum(f, 20.0) * LOG2E)
                n = e * (e + 2.0)
                put(kind, "act", off, (f * (n * pltpu.reciprocal(n + 2.0, approx=True))).astype(bf16))
            elif kind == "down":
                out = get("h", off) + matmul(get("act", off), weights(w2_v), 22)
                out_v[pl.ds(first_row(base + off), R), :] = out.astype(bf16)
            else:
                raise ValueError(kind)

    run_region("pro", _PROLOGUE, 0)

    def loop_step(k, carry):
        run_region("body", _BODY, _LOOP_BASES[0] + 2 * k)
        return carry

    jax.lax.fori_loop(0, len(_LOOP_BASES), loop_step, None)
    run_region("epi", _EPILOGUE, 0)

    for kind, off, opt in _EPILOGUE:
        if kind == "send":
            out_copy(off, opt).wait()
    for kind, off, opt in _BODY:
        if kind == "send":
            for b in _LOOP_BASES:
                out_copy(b + off, opt).wait()


def kernel(A_x, A_wqkv, A_wo, B_x, B_w1, B_b1, B_w2):
    del B_x
    hbm = pl.BlockSpec(memory_space=pltpu.HBM)
    out = pl.pallas_call(
        _body,
        in_specs=[hbm] * 6,
        out_specs=hbm,
        out_shape=jax.ShapeDtypeStruct((S, D), bf16),
        scratch_shapes=[
            pltpu.VMEM((S, D), bf16),
            pltpu.VMEM((3, D, D), bf16),
            pltpu.VMEM((3, D // 2, D), u32),
            pltpu.VMEM((D, D), bf16),
            pltpu.VMEM((D // 2, D), u32),
            pltpu.VMEM((F, D), bf16),
            pltpu.VMEM((F, D), bf16),
            pltpu.VMEM((F,), bf16),
            pltpu.VMEM((8, F), f32),
            pltpu.VMEM((S, D), bf16),
            pltpu.VMEM((NT, 4, HALO + R, 128), f32),
            pltpu.VMEM((NT, 4, HALO + R, 128), f32),
            pltpu.VMEM((NT, R, D), f32),
            pltpu.VMEM((NT, R, D), f32),
            pltpu.VMEM((NT, RW, D), u32),
            pltpu.VMEM((NT, RW, F), u32),
            pltpu.SemaphoreType.DMA((len(_DMA_GROUPS),)),
            pltpu.SemaphoreType.DMA((1,)),
        ],
        compiler_params=pltpu.CompilerParams(vmem_limit_bytes=100 * 1024 * 1024),
    )(A_x.reshape(S, D), A_wqkv, A_wo, B_w1.T, B_b1, B_w2)
    return out.reshape(1, S, D)


@jax.jit
def pallas_sequential_preLN__sliding_local_dilated__dense_activation_mish__prompt_kernel(
    A_x: jax.Array,
    A_wqkv: jax.Array,
    A_wo: jax.Array,
    B_x: jax.Array,
    B_w1: jax.Array,
    B_b1: jax.Array,
    B_w2: jax.Array,
):
    return kernel(A_x, A_wqkv, A_wo, B_x, B_w1, B_b1, B_w2)
```

```python
import jax
import jax.numpy as jnp
import jax.experimental.pallas as pl
import jax.experimental.pallas.tpu as pltpu

S, D, F = 2048, 512, 1376
WINDOW, DILATION = 8, 2
R = 256
RW = R // 2
NT = S // R
G = 8
NG = R // G
HALO = 16
PB = 32
LOG2E = 1.4426950408889634
QK_SCALE = 0.25 * LOG2E
MASKED = -1e9 * LOG2E
f32, bf16, u32 = jnp.float32, jnp.bfloat16, jnp.uint32

_DMA_GROUPS = (("x0",), ("wq",), ("x12",), ("wk", "wv"), ("wo", "b1", "w1"), ("w2", "x37"))


def _att(t, chain, lag, tie, span, skip, pin=False):
    return ("att", t, dict(chain=chain, lag=lag, tie=tie, span=span, skip=skip, pin=pin))


_PROLOGUE = (
    ("wait", 0, None), ("ln", 0, None),
    ("wait", 1, None), ("perm_qkv", 0, None), ("q", 0, (0, 2)),
    ("wait", 2, None), ("ln", 1, None), ("q", 0, (2, 4)), ("q", 1, (0, 4)), ("ln", 2, None), ("q", 2, (0, 3)),
    ("wait", 3, None), ("perm_qkv", 1, None), ("q", 2, (3, 4)), ("k", 0, (0, 4)),
    ("perm_qkv", 2, None), ("v", 0, (0, 4)), ("k", 1, (0, 4)),
    _att(0, 6, 2, 2, 85, 15), ("v", 1, (0, 3)),
    ("wait", 4, None), ("v", 1, (3, 4)), ("perm_wo", 0, None), ("o", 0, None), ("prep_b", 0, None),
    ("v", 2, (0, 3)), ("k", 2, (0, 4)),
    _att(1, 6, 1, 3, 90, 8), ("v", 2, (3, 4)), ("o", 1, None), ("up", 0, None), ("mish", 0, None),
    ("wait", 5, None),
)
_BODY = (
    ("ln", 1, None), ("down", -2, None), ("q", 1, (0, 4)), ("k", 1, (0, 4)),
    _att(0, 9, 2, 3, 98, 0), ("o", 0, None), ("v", 1, (0, 4)),
    ("ln", 2, None), ("q", 2, (0, 4)), ("up", -1, None), ("mish", -1, None), ("down", -1, None), ("k", 2, (0, 4)),
    _att(1, 6, 0, 4, 90, 0), ("o", 1, None), ("v", 2, (0, 4)), ("up", 0, None), ("mish", 0, None),
    ("send", -2, 2),
)
_EPILOGUE = (
    ("down", 4, None), ("ln", 7, None), ("q", 7, (0, 4)), ("k", 7, (0, 4)),
    _att(6, 10, 2, 3, 98, 0), ("o", 6, None), ("v", 7, (0, 4)), ("up", 5, None), ("mish", 5, None),
    _att(7, 9, 1, 2, 80, 8, pin=True), ("o", 7, None), ("down", 5, None),
    ("up", 6, None), ("mish", 6, None), ("down", 6, None), ("up", 7, None),
    ("send", 4, 3), ("mish", 7, None), ("down", 7, None), ("send", 7, 1),
)
_LOOP_BASES = (2, 4)

_READS = dict(q=("xn",), k=("xn",), v=("xn",), o=("ctx",), up=("hn",), mish=("f",), down=("act", "h"))
_WRITES = dict(ln=("xn",), att=("ctx",), o=("h", "hn"), up=("f",), mish=("act",))


def _values_crossing_regions():
    regions = [("pro", _PROLOGUE, 0)] + [("body", _BODY, b) for b in _LOOP_BASES] + [("epi", _EPILOGUE, 0)]
    made, keep = {}, set()
    for idx, (region, steps, base) in enumerate(regions):
        for kind, off, _ in steps:
            for name in _READS.get(kind, ()):
                src_idx, src = made[name, base + off]
                if src_idx != idx:
                    keep.add(src)
            for name in _WRITES.get(kind, ()):
                made[name, base + off] = (idx, (region, kind, off, name))
    return frozenset(keep)


def _layernorm(x):
    m = jnp.mean(x, axis=-1, keepdims=True)
    c = x - m
    v = jnp.mean(c * c, axis=-1, keepdims=True)
    return c * jax.lax.rsqrt(v + 1e-5)


def _body(x_hbm, wqkv_hbm, wo_hbm, w1_hbm, b1_hbm, w2_hbm, out_hbm,
          x_v, wqkv_raw, wqkv_p, wo_raw, wo_p, w1_v, w2_v, b1_v, b1_f, out_v,
          k_s, v_s, q_s, h_s, hn_s, act_s, in_sem, out_sem):
    keep = _values_crossing_regions()
    stash = dict(h=h_s, hn=hn_s, act=act_s)

    def x_copy(t0, t1, sem):
        rows = pl.ds(t0 * R, (t1 - t0) * R)
        return pltpu.make_async_copy(x_hbm.at[rows, :], x_v.at[rows, :], sem)

    sem_of = {name: in_sem.at[i] for i, group in enumerate(_DMA_GROUPS) for name in group}
    copies = {
        "x0": x_copy(0, 1, sem_of["x0"]),
        "wq": pltpu.make_async_copy(wqkv_hbm.at[:, pl.ds(0, D)], wqkv_raw.at[0], sem_of["wq"]),
        "wk": pltpu.make_async_copy(wqkv_hbm.at[:, pl.ds(D, D)], wqkv_raw.at[1], sem_of["wk"]),
        "wv": pltpu.make_async_copy(wqkv_hbm.at[:, pl.ds(2 * D, D)], wqkv_raw.at[2], sem_of["wv"]),
        "wo": pltpu.make_async_copy(wo_hbm, wo_raw, sem_of["wo"]),
        "b1": pltpu.make_async_copy(b1_hbm, b1_v, sem_of["b1"]),
        "x12": x_copy(1, 3, sem_of["x12"]),
        "w1": pltpu.make_async_copy(w1_hbm, w1_v, sem_of["w1"]),
        "w2": pltpu.make_async_copy(w2_hbm, w2_v, sem_of["w2"]),
        "x37": x_copy(3, NT, sem_of["x37"]),
    }
    for group in _DMA_GROUPS:
        for name in group:
            copies[name].start()

    def out_copy(t0, tiles):
        rows = pl.ds(t0 * R, tiles * R)
        return pltpu.make_async_copy(out_v.at[rows, :], out_hbm.at[rows, :], out_sem.at[0])

    lane = jax.lax.broadcasted_iota(jnp.int32, (PB, 128), 1)
    lane_grp = (lane % 16) // 4
    lane_head = lane % 32

    def perm_qkv(p):
        src = wqkv_raw.at[p]
        idx = [(lane_head % 8) * 16 + 4 * ((lane_head // 8 + j) % 4) + lane // 32 for j in range(4)]
        for r0 in range(0, D // 2, PB):
            cols = [pltpu.bitcast(src[2 * r0:2 * (r0 + PB), i * 128:(i + 1) * 128], u32) for i in range(4)]
            for j in range(4):
                merged = cols[0]
                for i in range(1, 4):
                    merged = jnp.where(lane_grp == (i + j) % 4, cols[i], merged)
                wqkv_p[p, r0:r0 + PB, j * 128:(j + 1) * 128] = jnp.take_along_axis(merged, idx[j], axis=1)

    def perm_wo():
        sub = jax.lax.broadcasted_iota(jnp.int32, (8, 128), 0)

        def transpose8(xs):
            for b in (4, 2, 1):
                low = (sub & b) == 0
                ys = list(xs)
                for i in range(8):
                    if i & b == 0:
                        ys[i] = jnp.where(low, xs[i], pltpu.roll(xs[i + b], b, axis=0))
                        ys[i + b] = jnp.where(low, pltpu.roll(xs[i], 8 - b, axis=0), xs[i + b])
                xs = ys
            return xs

        for j in range(4):
            for a0 in (0, 8):
                even, odd = [], []
                for a in range(a0, a0 + 8):
                    lo = pltpu.bitcast(wo_raw[(2 * a) * 16:(2 * a) * 16 + 16, j * 128:(j + 1) * 128], u32)
                    hi = pltpu.bitcast(wo_raw[(2 * a + 1) * 16:(2 * a + 1) * 16 + 16, j * 128:(j + 1) * 128], u32)
                    even.append((lo & jnp.uint32(0xFFFF)) | (hi << 16))
                    odd.append((lo >> 16) | (hi & jnp.uint32(0xFFFF0000)))
                even, odd = transpose8(even), transpose8(odd)
                by_d = [None] * 16
                for m in range(8):
                    by_d[2 * m], by_d[2 * m + 1] = even[m], odd[m]
                i0 = a0 // 4
                for jj in range(4):
                    for g in range(4):
                        first = by_d[4 * ((i0 + jj) % 4) + g]
                        second = by_d[4 * ((i0 + 1 + jj) % 4) + g]
                        r = jj * 64 + g * 16 + a0
                        wo_p[r:r + 8, j * 128:(j + 1) * 128] = jnp.where(sub < 4, first, second)

    def prep_b():
        b1_f[...] = jnp.broadcast_to(b1_v[...].astype(f32)[None, :], (8, F))

    def weights(ref):
        return ref[...] if ref.dtype == bf16 else pltpu.bitcast(ref[...], bf16)

    def run_region(region, steps, base):
        local = {}
        matmuls = []
        att_parts = [None]

        def put(kind, name, off, val):
            local[name, off] = val
            if (region, kind, off, name) in keep:
                stash[name][base + off] = val if name == "h" else pltpu.bitcast(val, u32)

        def get(name, off):
            if (name, off) in local:
                return local[name, off]
            val = stash[name][base + off]
            return val if name == "h" else pltpu.bitcast(val, bf16)

        def matmul(lhs, rhs, cycles, transposed=False):
            dims = (((1,), (1 if transposed else 0,)), ((), ()))
            val = jax.lax.dot_general(lhs, rhs, dims, preferred_element_type=f32)
            matmuls.append((val, cycles))
            return val

        def first_row(t):
            return t * R if isinstance(t, int) else pl.multiple_of(t * R, R)

        def load_x(t):
            return x_v[pl.ds(first_row(t), R), :].astype(f32)

        def qkv_proj(kind, off, cols):
            t, (n0, n1), p = base + off, cols, "qkv".index(kind)
            first = isinstance(t, int) and t == 0
            last = isinstance(t, int) and t == NT - 1
            w = pltpu.bitcast(wqkv_p[p, :, n0 * 128:n1 * 128], bf16)
            val = matmul(get("xn", off), w, 8)
            if kind == "q":
                q_s[t, :, n0 * 128:n1 * 128] = val
                return
            dst = k_s if kind == "k" else v_s
            for j in range(n0, n1):
                col = val[:, (j - n0) * 128:(j - n0 + 1) * 128]
                dst[t, j, HALO:, :] = col
                if first:
                    dst[t, j, 0:HALO, :] = (jnp.zeros((HALO, 128), f32) if kind == "k"
                                            else jnp.broadcast_to(col[0:1, :], (HALO, 128)))
                if not last:
                    dst[t + 1, j, 0:HALO, :] = col[R - HALO:, :]

        def attention(off, opt):
            t = base + off
            first = isinstance(t, int) and t == 0
            stream, now = [], 0
            for val, cycles in matmuls[-opt["tie"]:]:
                for j in range(val.shape[1] // 128):
                    for r in range(R // 8):
                        stream.append((now, val, r, j))
                        now += cycles
            skip, span = opt["skip"] * now // 100, opt["span"] * now // 100
            release = []
            for g in range(NG):
                _, val, r, j = [e for e in stream if e[0] <= skip + g * span // NG][-1]
                release.append(val[r * 8:(r + 1) * 8, j * 128:(j + 1) * 128])

            denom, half, logits, ctx = [None] * NG, [None] * NG, [None] * NG, [None] * NG

            def products(g):
                r0 = g * G
                scale = jnp.full((G, 128), QK_SCALE, f32)
                if g >= opt["chain"]:
                    scale = jnp.minimum(scale, denom[g - opt["chain"]])
                gate = jnp.minimum(release[g], 0.0)
                if opt["pin"] and ("hn32", off - 1) in local:
                    gate = jnp.minimum(gate, local["hn32", off - 1][r0:r0 + 8, 0:128])
                scale = jnp.maximum(scale, gate)
                q = [q_s[t, r0:r0 + G, j * 128:(j + 1) * 128] * scale for j in range(4)]
                sums = []
                for w in range(WINDOW):
                    acc = None
                    for j in range(4):
                        prod = q[j] * k_s[t, j, pl.ds(HALO + r0 - w * DILATION, G), :]
                        acc = prod if acc is None else acc + prod
                    sums.append(acc)
                rolled = [pltpu.roll(s, 64, axis=1) for s in sums]
                half[g] = [s + r for s, r in zip(sums, rolled)]

            def finish_logits(g):
                r0 = g * G
                rolled = [pltpu.roll(s, 32, axis=1) for s in half[g]]
                full = [s + r for s, r in zip(half[g], rolled)]
                if first:
                    for w in range(WINDOW):
                        if r0 < w * DILATION:
                            pos = r0 + jax.lax.broadcasted_iota(jnp.int32, (G, 128), 0)
                            full[w] = jnp.where(pos >= w * DILATION, full[w], MASKED)
                logits[g] = full

            def softmax_values(g):
                r0 = g * G
                ls = logits[g]
                m = jnp.maximum(jnp.maximum(jnp.maximum(ls[0], ls[1]), jnp.maximum(ls[2], ls[3])),
                                jnp.maximum(jnp.maximum(ls[4], ls[5]), jnp.maximum(ls[6], ls[7])))
                es = [jnp.exp2(l - m) for l in ls]
                denom[g] = ((es[0] + es[1]) + (es[2] + es[3])) + ((es[4] + es[5]) + (es[6] + es[7]))
                acc = [None] * 4
                for w in range(WINDOW):
                    for j in range(4):
                        prod = es[w] * v_s[t, j, pl.ds(HALO + r0 - w * DILATION, G), :]
                        acc[j] = prod if acc[j] is None else acc[j] + prod
                inv = pltpu.reciprocal(denom[g], approx=True)
                ctx[g] = jnp.concatenate([a * inv for a in acc], axis=1)

            lag = opt["lag"]
            for i in range(NG + lag + 1):
                if i < NG:
                    products(i)
                if 0 <= i - lag < NG:
                    finish_logits(i - lag)
                if 0 <= i - lag - 1 < NG:
                    softmax_values(i - lag - 1)
            put("att", "ctx", off, jnp.concatenate(ctx, axis=0).astype(bf16))

        for kind, off, opt in steps:
            if kind == "wait":
                for name in _DMA_GROUPS[off]:
                    copies[name].wait()
            elif kind == "send":
                out_copy(base + off, opt).start()
            elif kind == "perm_qkv":
                perm_qkv(off)
            elif kind == "perm_wo":
                perm_wo()
            elif kind == "prep_b":
                prep_b()
            elif kind == "ln":
                put(kind, "xn", off, _layernorm(load_x(base + off)).astype(bf16))
            elif kind in ("q", "k", "v"):
                qkv_proj(kind, off, opt)
            elif kind == "att":
                attention(off, opt)
            elif kind == "o":
                h = load_x(base + off) + matmul(get("ctx", off), weights(wo_p), 8)
                put(kind, "h", off, h)
                hn = _layernorm(h)
                local["hn32", off] = hn
                put(kind, "hn", off, hn.astype(bf16))
            elif kind == "up":
                put(kind, "f", off, matmul(get("hn", off), weights(w1_v), 8, transposed=True) + b1_f[0:1, :])
            elif kind == "mish":
                f = get("f", off)
                e = jnp.exp2(jnp.minimum(f, 20.0) * LOG2E)
                n = e * (e + 2.0)
                put(kind, "act", off, (f * (n * pltpu.reciprocal(n + 2.0, approx=True))).astype(bf16))
            elif kind == "down":
                out = get("h", off) + matmul(get("act", off), weights(w2_v), 22)
                out_v[pl.ds(first_row(base + off), R), :] = out.astype(bf16)
            else:
                raise ValueError(kind)

    run_region("pro", _PROLOGUE, 0)

    def loop_step(k, carry):
        run_region("body", _BODY, _LOOP_BASES[0] + 2 * k)
        return carry

    jax.lax.fori_loop(0, len(_LOOP_BASES), loop_step, None)
    run_region("epi", _EPILOGUE, 0)

    for kind, off, opt in _EPILOGUE:
        if kind == "send":
            out_copy(off, opt).wait()
    for kind, off, opt in _BODY:
        if kind == "send":
            for b in _LOOP_BASES:
                out_copy(b + off, opt).wait()


def kernel(A_x, A_wqkv, A_wo, B_x, B_w1, B_b1, B_w2):
    del B_x
    hbm = pl.BlockSpec(memory_space=pltpu.HBM)
    out = pl.pallas_call(
        _body,
        in_specs=[hbm] * 6,
        out_specs=hbm,
        out_shape=jax.ShapeDtypeStruct((S, D), bf16),
        scratch_shapes=[
            pltpu.VMEM((S, D), bf16),
            pltpu.VMEM((3, D, D), bf16),
            pltpu.VMEM((3, D // 2, D), u32),
            pltpu.VMEM((D, D), bf16),
            pltpu.VMEM((D // 2, D), u32),
            pltpu.VMEM((F, D), bf16),
            pltpu.VMEM((F, D), bf16),
            pltpu.VMEM((F,), bf16),
            pltpu.VMEM((8, F), f32),
            pltpu.VMEM((S, D), bf16),
            pltpu.VMEM((NT, 4, HALO + R, 128), f32),
            pltpu.VMEM((NT, 4, HALO + R, 128), f32),
            pltpu.VMEM((NT, R, D), f32),
            pltpu.VMEM((NT, R, D), f32),
            pltpu.VMEM((NT, RW, D), u32),
            pltpu.VMEM((NT, RW, F), u32),
            pltpu.SemaphoreType.DMA((len(_DMA_GROUPS),)),
            pltpu.SemaphoreType.DMA((1,)),
        ],
        compiler_params=pltpu.CompilerParams(vmem_limit_bytes=100 * 1024 * 1024),
    )(A_x.reshape(S, D), A_wqkv, A_wo, B_w1.T, B_b1, B_w2)
    return out.reshape(1, S, D)


@jax.jit
def pallas_sequential_preLN__sliding_local_dilated__dense_activation_mish__prompt_kernel(
    A_x: jax.Array,
    A_wqkv: jax.Array,
    A_wo: jax.Array,
    B_x: jax.Array,
    B_w1: jax.Array,
    B_b1: jax.Array,
    B_w2: jax.Array,
):
    return kernel(A_x, A_wqkv, A_wo, B_x, B_w1, B_b1, B_w2)
```
